```python
import os as _os
_os.environ.setdefault("JAX_PLATFORMS", "cpu")
import jax
import jax.numpy as jnp

def _softmax(x, axis=-1):
    return jax.nn.softmax(x, axis=axis)
def _gelu(x):
    return jax.nn.gelu(x, approximate=True)
def _silu(x):
    return jax.nn.silu(x)
def _sigmoid(x):
    return jax.nn.sigmoid(x)
def _layernorm(x, axis=-1, eps=1e-5):
    m = jnp.mean(x, axis=axis, keepdims=True)
    v = jnp.var(x, axis=axis, keepdims=True)
    return (x - m) / jnp.sqrt(v + eps)
def _scatter_add(tgt, idx, src, axis=0):
    return tgt.at[idx].add(src)
def _segment_sum(src, seg, n):
    return jax.ops.segment_sum(src, seg, n)
class _Rng:
    def __init__(self, key):
        self._k = key
    def _next(self):
        self._k, sub = jax.random.split(self._k)
        return sub
    def normal(self, shape):
        return jax.random.normal(self._next(), shape, dtype=jnp.bfloat16)
    def randint(self, lo, hi, shape):
        return jax.random.randint(self._next(), shape, lo, hi, dtype=jnp.int32)
    def uniform(self, shape, lo=0.0, hi=1.0):
        return jax.random.uniform(self._next(), shape, jnp.bfloat16, lo, hi)
    def permutation(self, n):
        return jax.random.permutation(self._next(), n)


kernel_name = 'parallel_sum__sliding_block_cached__dense_activation_mish__decode'

def setup_inputs():
    _rng = _Rng(jax.random.key(int.from_bytes(__import__("os").urandom(4), "little")))
    _w = (lambda a: (lambda t: t.astype(jnp.bfloat16) if jnp.issubdtype(t.dtype, jnp.floating) else t)(jnp.asarray(a)))
    def _A_setup():
        B, Sq, D = 2, 1, 512
        Hq, Hkv, Sk, Dh = 32, 8, 32768, 128
        assert Hq % Hkv == 0, (Hq, Hkv)
        return {
            "x": _w((lambda *s: _rng.normal(s) * 0.05)(B, Sq, D)),
            "k_cache": _w((lambda *s: _rng.normal(s) * 0.8)(B, Hkv, Sk, Dh)),
            "v_cache": _w((lambda *s: _rng.normal(s) * 0.8)(B, Hkv, Sk, Dh)),
            "wq": _w((lambda *s: _rng.normal(s) * 0.8)(D, Hq * Dh) * (D ** -0.5)),
            "wo": _w((lambda *s: _rng.normal(s) * 0.8)(Hq * Dh, D) * ((Hq * Dh) ** -0.5)),
        }
    _A_in = _A_setup()

    def _B_setup():
        B, S, D, F = 2, 1, 512, 1792
        return {
            "x": _w((lambda *s: _rng.normal(s) * 0.05)(B, S, D)),
            "w1": _w((lambda *s: _rng.normal(s) * 0.4)(D, F) * (D ** -0.5)),
            "b1": _w((lambda *s: _rng.normal(s) * 0.05)(F)),
            "w2": _w((lambda *s: _rng.normal(s) * 0.05)(F, D) * (F ** -0.5)),
        }
    _B_in = _B_setup()

    return {
        "A_x": _A_in["x"],
        "A_k_cache": _A_in["k_cache"],
        "A_v_cache": _A_in["v_cache"],
        "A_wq": _A_in["wq"],
        "A_wo": _A_in["wo"],
        "B_x": _B_in["x"],
        "B_w1": _B_in["w1"],
        "B_b1": _B_in["b1"],
        "B_w2": _B_in["w2"],
    }

def reference(A_x, A_k_cache, A_v_cache, A_wq, A_wo, B_x, B_w1, B_b1, B_w2):
    def _A_ref(x, k_cache, v_cache, wq, wo):
        B, Sq, D = x.shape
        Hq, Dh = 32, 128
        Hkv, Sk = k_cache.shape[1], k_cache.shape[2]
        W = min(4096, max(256, Sk // 4))
        rep = Hq // Hkv
        q = (lambda x, *d: x.transpose(*d))((x @ wq).reshape(B, Sq, Hq, Dh), 0, 2, 1, 3)
        k = jnp.repeat(k_cache[:, :, Sk - W:, :], rep, axis=1)
        v = jnp.repeat(v_cache[:, :, Sk - W:, :], rep, axis=1)
        scores = jnp.einsum("bhqd,bhkd->bhqk", q, k) * (Dh ** -0.5)
        p = _softmax(scores, axis=-1)
        o = jnp.einsum("bhqk,bhkd->bhqd", p, v)
        return (lambda x, *d: x.transpose(*d))(o, 0, 2, 1, 3).reshape(B, Sq, Hq * Dh) @ wo

    def _B_ref(x, w1, b1, w2):
        h = jnp.einsum("bsd,df->bsf", x, w1) + b1
        sp = jnp.log1p(jnp.exp(-jnp.abs(h))) + jnp.where(h > 0, h, jnp.zeros_like(h))
        act = h * jnp.tanh(sp)
        return jnp.einsum("bsf,fd->bsd", act, w2)

    x = A_x
    xn = _layernorm(x, axis=-1)
    return x + _A_ref(xn, A_k_cache, A_v_cache, A_wq, A_wo) + _B_ref(xn, B_w1, B_b1, B_w2)
```

```python
import jax
import jax.numpy as jnp
from jax import lax
import jax.experimental.pallas as pl
import jax.experimental.pallas.tpu as pltpu

HQ, DH = 32, 128
F32, BF16 = jnp.float32, jnp.bfloat16
WO_SPLITS = (3584, 384, 128)


@jax.jit
def pallas_parallel_sum__sliding_block_cached__dense_activation_mish__decode_kernel(
    A_x: jax.Array,
    A_k_cache: jax.Array,
    A_v_cache: jax.Array,
    A_wq: jax.Array,
    A_wo: jax.Array,
    B_x: jax.Array,
    B_w1: jax.Array,
    B_b1: jax.Array,
    B_w2: jax.Array,
):
    del B_x
    B, Sq, D = A_x.shape
    Hkv, Sk = A_k_cache.shape[1], A_k_cache.shape[2]
    W = min(4096, max(256, Sk // 4))
    rep = HQ // Hkv
    F = B_w1.shape[1]
    R = B * rep
    assert Sq == 1 and B == 2 and R == 8 and sum(WO_SPLITS) == HQ * DH
    GW = rep * DH

    def kernel(x_h, k_h, v_h, wq_h, wo_h, w1_h, b1_h, w2_h, o_ref,
               xb, kb, vb, wqb, wob, w1b, b1b, w2b, qb, lb, sem):
        def kcopy(g):
            return pltpu.make_async_copy(k_h.at[:, g, pl.ds(Sk - W, W)], kb.at[g], sem.at[0])

        def vcopy(g):
            return pltpu.make_async_copy(v_h.at[:, g, pl.ds(Sk - W, W)], vb.at[g], sem.at[1])

        head = [pltpu.make_async_copy(wq_h, wqb, sem.at[0]),
                pltpu.make_async_copy(x_h, xb, sem.at[0])]
        ffn = [pltpu.make_async_copy(w1_h, w1b, sem.at[1]),
               pltpu.make_async_copy(b1_h, b1b, sem.at[1]),
               pltpu.make_async_copy(w2_h, w2b, sem.at[1])]
        tail = []
        s0 = 0
        for i, n in enumerate(WO_SPLITS):
            tail.append((s0, n, pltpu.make_async_copy(
                wo_h.at[pl.ds(s0, n)], wob.at[pl.ds(s0, n)], sem.at[i])))
            s0 += n

        for c in head + ffn:
            c.start()

        row = lax.broadcasted_iota(jnp.int32, (R, DH), 0)
        for c in head:
            c.wait()
        kcopy(0).start()

        x = xb[...].astype(F32)
        mu = jnp.mean(x, axis=-1, keepdims=True)
        xc = x - mu
        var = jnp.mean(xc * xc, axis=-1, keepdims=True)
        xn = xc / jnp.sqrt(var + 1e-5)
        rowd = lax.broadcasted_iota(jnp.int32, (R, D), 0)
        xr = jnp.where(rowd < rep, xn[0:1], xn[1:2]).astype(BF16)

        for g in range(Hkv):
            qf = jnp.dot(xr, wqb[:, g * GW:(g + 1) * GW], preferred_element_type=F32)
            q = qf[:, 0:DH]
            for r in range(1, rep):
                q = jnp.where(row % rep == r, qf[:, r * DH:(r + 1) * DH], q)
            qb[g] = q

        for c in ffn:
            c.wait()
        vcopy(0).start()

        h = jnp.dot(xr, w1b[...], preferred_element_type=F32)
        b1 = b1b[...].astype(F32)
        bias = jnp.concatenate([b1[j:j + 1] for j in range(F // 128)], axis=1)
        h = h + bias
        sp = jnp.log1p(jnp.exp(-jnp.abs(h))) + jnp.where(h > 0, h, 0.0)
        act = h * jnp.tanh(sp)
        y_ffn = jnp.dot(act.astype(BF16), w2b[...], preferred_element_type=F32)

        nt = (((1,), (1,)), ((), ()))

        def body(g, carry):
            kcopy(g).wait()

            @pl.when(g + 1 < Hkv)
            def _():
                kcopy(g + 1).start()

            @pl.when(g + 1 == Hkv)
            def _():
                tail[0][2].start()

            q = qb[g].astype(BF16)
            s0_ = lax.dot_general(q, kb[g, 0], nt, preferred_element_type=F32)
            s1_ = lax.dot_general(q, kb[g, 1], nt, preferred_element_type=F32)
            roww = lax.broadcasted_iota(jnp.int32, (R, W), 0)
            s = jnp.where(roww < rep, s0_, s1_) * (DH ** -0.5)
            m = jnp.max(s, axis=-1, keepdims=True)
            p = jnp.exp(s - m)
            l = jnp.sum(p, axis=-1, keepdims=True)
            pb = p.astype(BF16)

            vcopy(g).wait()

            @pl.when(g + 1 < Hkv)
            def _():
                vcopy(g + 1).start()

            @pl.when(g + 1 == Hkv)
            def _():
                for t in tail[1:]:
                    t[2].start()

            o0 = jnp.dot(pb, vb[g, 0], preferred_element_type=F32)
            o1 = jnp.dot(pb, vb[g, 1], preferred_element_type=F32)
            o = jnp.where(row < rep, o0, o1) / l
            lb[g] = o
            return carry

        lax.fori_loop(0, Hkv, body, 0)

        pieces = []
        for g in range(Hkv):
            o = lb[g]
            for r in range(rep):
                pieces.append(jnp.where(row % rep == r, o, 0.0).astype(BF16))
        y = jnp.where(rowd % rep == 0, y_ffn, 0.0)
        for s0, n, c in tail:
            lhs = jnp.concatenate(pieces[s0 // DH:(s0 + n) // DH], axis=1)
            c.wait()
            y = y + jnp.dot(lhs, wob[pl.ds(s0, n), :], preferred_element_type=F32)
        y0 = jnp.sum(jnp.where(rowd < rep, y, 0.0), axis=0, keepdims=True)
        y1 = jnp.sum(jnp.where(rowd >= rep, y, 0.0), axis=0, keepdims=True)
        o_ref[...] = (x + jnp.concatenate([y0, y1], axis=0)).astype(o_ref.dtype)

    hbm = pl.BlockSpec(memory_space=pltpu.HBM)
    out = pl.pallas_call(
        kernel,
        in_specs=[hbm] * 8,
        out_specs=pl.BlockSpec(memory_space=pltpu.VMEM),
        out_shape=jax.ShapeDtypeStruct((B, D), A_x.dtype),
        scratch_shapes=[
            pltpu.VMEM((B, D), BF16),
            pltpu.VMEM((Hkv, B, W, DH), BF16),
            pltpu.VMEM((Hkv, B, W, DH), BF16),
            pltpu.VMEM(A_wq.shape, BF16),
            pltpu.VMEM(A_wo.shape, BF16),
            pltpu.VMEM(B_w1.shape, BF16),
            pltpu.VMEM((F // 128, 128), BF16),
            pltpu.VMEM(B_w2.shape, BF16),
            pltpu.VMEM((Hkv, R, DH), F32),
            pltpu.VMEM((Hkv, R, DH), F32),
            pltpu.SemaphoreType.DMA((max(2, len(WO_SPLITS)),)),
        ],
        compiler_params=pltpu.CompilerParams(vmem_limit_bytes=64 * 1024 * 1024),
    )(A_x.reshape(B, D), A_k_cache, A_v_cache, A_wq, A_wo, B_w1,
      B_b1.reshape(F // 128, 128), B_w2)
    return out.reshape(B, Sq, D)
```

```python
import jax
import jax.numpy as jnp
from jax import lax
import jax.experimental.pallas as pl
import jax.experimental.pallas.tpu as pltpu

HQ, DH = 32, 128
EPS = 1e-5
F32, BF16 = jnp.float32, jnp.bfloat16


@jax.jit
def pallas_parallel_sum__sliding_block_cached__dense_activation_mish__decode_kernel(
    A_x: jax.Array,
    A_k_cache: jax.Array,
    A_v_cache: jax.Array,
    A_wq: jax.Array,
    A_wo: jax.Array,
    B_x: jax.Array,
    B_w1: jax.Array,
    B_b1: jax.Array,
    B_w2: jax.Array,
):
    del B_x
    B, Sq, D = A_x.shape
    Hkv, Sk = A_k_cache.shape[1], A_k_cache.shape[2]
    F = B_w1.shape[1]
    W = min(4096, max(256, Sk // 4))
    rep = HQ // Hkv
    R = B * rep
    GW = rep * DH
    G1 = Hkv - 1
    LAST = HQ * DH - DH
    assert Sq == 1 and B == 2 and R == 8 and Hkv % 2 == 0

    def kernel(x_h, k_h, v_h, wq_h, wo_h, w1_h, b1_h, w2_h, o_ref,
               xb, kb, vb, wqb, wob, w1b, b1b, w2b, qb, ob, cb):
        row = lax.broadcasted_iota(jnp.int32, (R, DH), 0)
        rowd = lax.broadcasted_iota(jnp.int32, (R, D), 0)

        def block_diag(o):
            return jnp.concatenate(
                [jnp.where(row // B == r, o, 0.0).astype(BF16) for r in range(rep)], axis=1)

        def project(g, y):
            w = wob[pl.ds(pl.multiple_of(g * GW, GW), GW), :]
            return y + jnp.dot(block_diag(ob[g]), w, preferred_element_type=F32)

        def project_last_head(lo, hi, acc):
            acc = list(acc)
            for i in range(lo, hi, 2 * R):
                w = wob[pl.ds(LAST + i, 2 * R), :].astype(F32)
                for b in range(B):
                    c = cb[b, pl.ds(i, 2 * R), :]
                    t = w * jnp.concatenate([c] * (D // DH), axis=1)
                    t = t[:R] + t[R:]
                    acc[b] = t if acc[b] is None else acc[b] + t
            return acc

        def stream(sem0, sem1, sem2):
            def k_copy(g):
                return pltpu.make_async_copy(k_h.at[:, g, pl.ds(Sk - W, W)], kb.at[g], sem0)

            def v_copy(g):
                return pltpu.make_async_copy(v_h.at[:, g, pl.ds(Sk - W, W)], vb.at[g], sem1)

            def wo_rows(start, size, sem):
                return pltpu.make_async_copy(
                    wo_h.at[pl.ds(start, size)], wob.at[pl.ds(start, size)], sem)

            def wo_copy(g, sem):
                return wo_rows(pl.multiple_of(g * GW, GW), GW, sem)

            head = [pltpu.make_async_copy(wq_h, wqb, sem0),
                    pltpu.make_async_copy(x_h, xb, sem0)]
            ffn = [pltpu.make_async_copy(w1_h, w1b, sem1),
                   pltpu.make_async_copy(b1_h, b1b, sem1),
                   pltpu.make_async_copy(w2_h, w2b, sem1)]
            tail0 = wo_rows(G1 * GW, GW - DH, sem1)
            tail1 = wo_rows(LAST, DH // 2, sem0)
            tail2 = wo_rows(LAST + DH // 2, DH // 2, sem2)

            for c in head + ffn:
                c.start()

            for c in head:
                c.wait()
            k_copy(0).start()
            x = xb[...].astype(F32)
            xc = x - jnp.mean(x, axis=-1, keepdims=True)
            var = jnp.mean(xc * xc, axis=-1, keepdims=True)
            xn = xc / jnp.sqrt(var + EPS)
            xr = jnp.where(rowd % B == 0, xn[0:1], xn[1:2]).astype(BF16)
            for g in range(Hkv):
                qf = jnp.dot(xr, wqb[:, g * GW:(g + 1) * GW], preferred_element_type=F32)
                q = qf[:, :DH]
                for r in range(1, rep):
                    q = jnp.where(row // B == r, qf[:, r * DH:(r + 1) * DH], q)
                qb[g] = q

            for c in ffn:
                c.wait()
            v_copy(0).start()
            b1 = b1b[...].astype(F32)
            bias = jnp.concatenate([b1[j:j + 1] for j in range(F // 128)], axis=1)
            h = jnp.dot(xr, w1b[...], preferred_element_type=F32) + bias
            sp = jnp.log1p(jnp.exp(-jnp.abs(h))) + jnp.where(h > 0, h, 0.0)
            act = h * jnp.tanh(sp)
            ffn_out = jnp.dot(act.astype(BF16), w2b[...], preferred_element_type=F32)
            y = jnp.where(rowd < B, ffn_out + jnp.where(rowd % B == 0, x[0:1], x[1:2]), 0.0)

            def attend(g, carry):
                k_copy(g).wait()

                @pl.when(g < G1)
                def _():
                    k_copy(g + 1).start()

                @pl.when(g == G1)
                def _():
                    wo_copy(0, sem0).start()

                q = qb[g].astype(BF16)
                nt = (((1,), (1,)), ((), ()))
                s0 = lax.dot_general(q, kb[g, 0], nt, preferred_element_type=F32)
                s1 = lax.dot_general(q, kb[g, 1], nt, preferred_element_type=F32)
                roww = lax.broadcasted_iota(jnp.int32, (R, W), 0)
                s = jnp.where(roww % B == 0, s0, s1) * (DH ** -0.5)
                p = jnp.exp(s - jnp.max(s, axis=-1, keepdims=True))
                l = jnp.sum(p, axis=-1, keepdims=True)
                p = p.astype(BF16)

                v_copy(g).wait()

                @pl.when(g < G1)
                def _():
                    v_copy(g + 1).start()

                @pl.when(g == G1)
                def _():
                    wo_copy(1, sem1).start()

                o0 = jnp.dot(p, vb[g, 0], preferred_element_type=F32)
                o1 = jnp.dot(p, vb[g, 1], preferred_element_type=F32)
                ob[g] = jnp.where(row % B == 0, o0, o1) / l
                return carry

            lax.fori_loop(0, Hkv, attend, 0)

            ot = jnp.transpose(jnp.concatenate([ob[G1]] * (DH // R), axis=0))
            for b in range(B):
                col = ot[:, R - B + b:R - B + b + 1].astype(BF16).astype(F32)
                cb[b] = jnp.broadcast_to(col, (DH, DH))

            def project_pair(i, y):
                g = 2 * i
                wo_copy(g, sem0).wait()
                wo_copy(g + 2, sem0).start()
                y = project(g, y)
                wo_copy(g + 1, sem1).wait()

                @pl.when(g + 3 < G1)
                def _():
                    wo_copy(g + 3, sem1).start()

                @pl.when(g + 3 == G1)
                def _():
                    tail0.start()

                return project(g + 1, y)

            y = lax.fori_loop(0, G1 // 2, project_pair, y)
            wo_copy(G1 - 1, sem0).wait()
            tail1.start()
            tail2.start()
            y = project(G1 - 1, y)
            lhs = block_diag(ob[G1])[:, :GW - DH]
            tail0.wait()
            y = y + jnp.dot(lhs, wob[pl.ds(G1 * GW, GW - DH), :], preferred_element_type=F32)
            tail1.wait()
            acc = project_last_head(0, DH // 2, [None] * B)
            tail2.wait()
            return y, acc

        y, acc = pl.run_scoped(stream, *[pltpu.SemaphoreType.DMA(())] * 3)
        acc = project_last_head(DH // 2, DH, acc)

        even = rowd % B == 0
        y = y + jnp.where(even, acc[0], acc[1]) + pltpu.roll(jnp.where(even, acc[1], acc[0]), 1, axis=0)
        y = y + pltpu.roll(y, 4, axis=0)
        y = y + pltpu.roll(y, 2, axis=0)
        o_ref[...] = y[:B].astype(o_ref.dtype)

    hbm = pl.BlockSpec(memory_space=pltpu.HBM)
    out = pl.pallas_call(
        kernel,
        in_specs=[hbm] * 8,
        out_specs=pl.BlockSpec(memory_space=pltpu.VMEM),
        out_shape=jax.ShapeDtypeStruct((B, D), A_x.dtype),
        scratch_shapes=[
            pltpu.VMEM((B, D), A_x.dtype),
            pltpu.VMEM((Hkv, B, W, DH), A_k_cache.dtype),
            pltpu.VMEM((Hkv, B, W, DH), A_v_cache.dtype),
            pltpu.VMEM(A_wq.shape, A_wq.dtype),
            pltpu.VMEM(A_wo.shape, A_wo.dtype),
            pltpu.VMEM(B_w1.shape, B_w1.dtype),
            pltpu.VMEM((F // 128, 128), B_b1.dtype),
            pltpu.VMEM(B_w2.shape, B_w2.dtype),
            pltpu.VMEM((Hkv, R, DH), F32),
            pltpu.VMEM((Hkv, R, DH), F32),
            pltpu.VMEM((B, DH, DH), F32),
        ],
        compiler_params=pltpu.CompilerParams(vmem_limit_bytes=64 * 1024 * 1024),
    )(A_x.reshape(B, D), A_k_cache, A_v_cache, A_wq, A_wo, B_w1,
      B_b1.reshape(F // 128, 128), B_w2)
    return out.reshape(B, Sq, D)
```
